```python
import os as _os
_os.environ.setdefault("JAX_PLATFORMS", "cpu")
import jax
import jax.numpy as jnp

def _softmax(x, axis=-1):
    return jax.nn.softmax(x, axis=axis)
def _gelu(x):
    return jax.nn.gelu(x, approximate=True)
def _silu(x):
    return jax.nn.silu(x)
def _sigmoid(x):
    return jax.nn.sigmoid(x)
def _layernorm(x, axis=-1, eps=1e-5):
    m = jnp.mean(x, axis=axis, keepdims=True)
    v = jnp.var(x, axis=axis, keepdims=True)
    return (x - m) / jnp.sqrt(v + eps)
def _scatter_add(tgt, idx, src, axis=0):
    return tgt.at[idx].add(src)
def _segment_sum(src, seg, n):
    return jax.ops.segment_sum(src, seg, n)
class _Rng:
    def __init__(self, key):
        self._k = key
    def _next(self):
        self._k, sub = jax.random.split(self._k)
        return sub
    def normal(self, shape):
        return jax.random.normal(self._next(), shape, dtype=jnp.bfloat16)
    def randint(self, lo, hi, shape):
        return jax.random.randint(self._next(), shape, lo, hi, dtype=jnp.int32)
    def uniform(self, shape, lo=0.0, hi=1.0):
        return jax.random.uniform(self._next(), shape, jnp.bfloat16, lo, hi)
    def permutation(self, n):
        return jax.random.permutation(self._next(), n)


kernel_name = 'interleave_layers__sliding_local_dilated__mixer_channel_mlp__prompt'

def setup_inputs():
    _rng = _Rng(jax.random.key(int.from_bytes(__import__("os").urandom(4), "little")))
    _w = (lambda a: (lambda t: t.astype(jnp.bfloat16) if jnp.issubdtype(t.dtype, jnp.floating) else t)(jnp.asarray(a)))
    def _A_setup():
        B, S, D = 1, 2048, 512
        return {
            "x": _w((lambda *s: _rng.normal(s) * 0.05)(B, S, D)),
            "wqkv": _w((lambda *s: _rng.normal(s) * 0.05)(D, 3 * D)),
            "wo": _w((lambda *s: _rng.normal(s) * 0.05)(D, D)),
        }
    _A_in = _A_setup()

    def _B_setup():
        B, S, D, F = 1, 2048, 512, 1376
        return {
            "x": _w((lambda *s: _rng.normal(s) * 0.05)(B, S, D)),
            "w1": _w((lambda *s: _rng.normal(s) * 0.4)(D, F) * (D ** -0.5)),
            "b1": _w((lambda *s: _rng.normal(s) * 0.4)(F)),
            "w2": _w((lambda *s: _rng.normal(s) * 0.4)(F, D) * (F ** -0.5)),
            "b2": _w((lambda *s: _rng.normal(s) * 0.4)(D)),
        }
    _B_in = _B_setup()

    return {
        "A_x": _A_in["x"],
        "A_wqkv": _A_in["wqkv"],
        "A_wo": _A_in["wo"],
        "B_x": _B_in["x"],
        "B_w1": _B_in["w1"],
        "B_b1": _B_in["b1"],
        "B_w2": _B_in["w2"],
        "B_b2": _B_in["b2"],
    }

def reference(A_x, A_wqkv, A_wo, B_x, B_w1, B_b1, B_w2, B_b2):
    def _A_ref(x, wqkv, wo):
        B, S, D = x.shape
        H = 32; Dh = D // H
        W, dil = 8, 2
        qkv = (lambda x, *d: x.transpose(*d))((x @ wqkv).reshape(B, S, 3, H, Dh), 2, 0, 3, 1, 4)
        q, k, v = qkv[0], qkv[1], qkv[2]
        scale = Dh ** -0.5
        pos = jnp.arange(S)
        off = jnp.arange(W) * dil
        idx = pos[:, None] - off[None, :]
        mask = idx >= 0
        idx_c = jnp.where(mask, idx, 0).reshape(-1)
        kg = k[:, :, idx_c, :].reshape(B, H, S, W, Dh)
        vg = v[:, :, idx_c, :].reshape(B, H, S, W, Dh)
        logits = jnp.einsum("bhsd,bhswd->bhsw", q, kg) * scale
        logits = jnp.where(mask[None, None, :, :], logits, -1e9)
        attn = _softmax(logits, axis=-1)
        o = jnp.einsum("bhsw,bhswd->bhsd", attn, vg)
        return (lambda x, *d: x.transpose(*d))(o, 0, 2, 1, 3).reshape(B, S, D) @ wo

    def _B_ref(x, w1, b1, w2, b2):
        y = _layernorm(x, axis=-1)
        h = _gelu(jnp.einsum("bsd,df->bsf", y, w1) + b1)
        return jnp.einsum("bsf,fd->bsd", h, w2) + b2

    x = A_x
    x = x + _A_ref(_layernorm(x, axis=-1), A_wqkv, A_wo)
    x = x + _B_ref(_layernorm(x, axis=-1), B_w1, B_b1, B_w2, B_b2)
    x = x + _A_ref(_layernorm(x, axis=-1), A_wqkv, A_wo)
    x = x + _B_ref(_layernorm(x, axis=-1), B_w1, B_b1, B_w2, B_b2)
    return x
```

```python
import functools
import jax
import jax.numpy as jnp
import jax.experimental.pallas as pl
import jax.experimental.pallas.tpu as pltpu

S, D, F = 2048, 512, 1376
H, DH, W, DIL = 32, 16, 8, 2
T = int("512")
TS = int("128")
RC = int("16")
LC = int("32")
CATT = int("160")
CLN = int("100")
GW = int("50")
ORDER = "L1_Q0_L2_Q1_O0_L3_Q2_W_A0_O1_B0_A1_O2_Q3_q0_B1_A2_O3_o0_q1_B2_A3_a0_o1_q2_B3_b0_a1_o2_q3_b1_a2_o3_N_b2_a3_b3"
B1D = int("1")
NS = T // TS
NB = S // T
HALO = 16
EPS = 1e-5
NC = D // 128
f32 = jnp.float32
bf16 = jnp.bfloat16
u32 = jnp.uint32
NT = (((1,), (1,)), ((), ()))


def _ln(x):
    m = jnp.mean(x, axis=-1, keepdims=True)
    xc = x - m
    v = jnp.mean(xc * xc, axis=-1, keepdims=True)
    return xc * jax.lax.rsqrt(v + EPS)


def _gelu(x):
    c = 0.7978845608028654
    return 0.5 * x * (1.0 + jnp.tanh(c * (x + 0.044715 * (x * x * x))))


def _pack(x):
    return pltpu.bitcast(x.astype(bf16), u32)


def _unpack(x):
    return pltpu.bitcast(x, bf16)


def kernel(x_hbm, wqkv_hbm, wo_hbm, w1_hbm, b1_hbm, w2_hbm, b2_hbm, o_hbm,
           b1_ref, b2_ref, xf_ref, xr_ref, ob_ref, wraw_ref, woraw_ref, wt_ref, wop_ref, w1_ref, w2_ref,
           xs_ref, xn_ref, q_ref, kv_ref, a_ref, g_ref,
           sem_w):
    blk = pl.program_id(0)
    row0 = pl.multiple_of(blk * T, T)

    def xf_copy(b):
        return pltpu.make_async_copy(x_hbm.at[pl.ds(b * T, TS), :], xf_ref, sem_w.at[9])

    def xr_copy(b):
        return pltpu.make_async_copy(x_hbm.at[pl.ds(b * T + TS, T - TS), :], xr_ref,
                                     sem_w.at[10])

    def o_copy(b):
        return pltpu.make_async_copy(ob_ref, o_hbm.at[pl.ds(b * T, T), :], sem_w.at[11])

    def wqkv_copy(j):
        return pltpu.make_async_copy(wqkv_hbm.at[:, pl.ds(j * 256, 256)], wraw_ref.at[:, pl.ds(j * 256, 256)],
                                     sem_w.at[j])

    wo_copy = pltpu.make_async_copy(wo_hbm, woraw_ref, sem_w.at[6])
    w1_copy = pltpu.make_async_copy(w1_hbm, w1_ref, sem_w.at[7])
    w2_copy = pltpu.make_async_copy(w2_hbm, w2_ref, sem_w.at[8])
    b1_copy = pltpu.make_async_copy(b1_hbm, b1_ref, sem_w.at[12])
    b2_copy = pltpu.make_async_copy(b2_hbm, b2_ref, sem_w.at[13])

    def rows(s):
        return slice(s * TS, (s + 1) * TS)

    def hrows(s):
        return slice(s * TS // 2, (s + 1) * TS // 2)

    def ln1_in(base, s):
        for r0 in range(s * TS, (s + 1) * TS, LC):
            x = (xf_ref[r0:r0 + LC, :] if s == 0 else xr_ref[r0 - TS:r0 - TS + LC, :]).astype(f32)
            xs_ref[r0:r0 + LC, :] = x
            xn_ref[r0 // 2:(r0 + LC) // 2, :] = _pack(_ln(x))
            yield CLN

    @pl.when(blk == 0)
    def _():
        xf_copy(0).start()
        for j in range(4):
            wqkv_copy(j).start()
        wo_copy.start()
        for j in range(4, 6):
            wqkv_copy(j).start()
        xr_copy(0).start()
        b1_copy.start()
        b2_copy.start()
        w1_copy.start()
        w2_copy.start()
        kv_ref[:, :, T:T + HALO, :] = jnp.zeros((2, 2 * NC, HALO, 128), f32)
        rho = jax.lax.broadcasted_iota(jnp.int32, (128, 128), 0)
        col = jax.lax.broadcasted_iota(jnp.int32, (128, 128), 1)
        hit = rho == (col % DH) * 8 + col // DH
        perm = jnp.where(hit, 1.0, 0.0).astype(bf16)
        perm_q = jnp.where(hit, DH ** -0.5, 0.0).astype(bf16)
        xf_copy(0).wait()
        list(ln1_in(0, 0))
        for j in range(6):
            if j == 4:
                wo_copy.wait()
                for pair in range(2):
                    o = []
                    for c in range(2):
                        wj = woraw_ref[(2 * pair + c) * 128:(2 * pair + c + 1) * 128, :]
                        o.append(jnp.dot(perm, wj, preferred_element_type=f32).reshape(DH, 8, D))
                    z = jnp.concatenate(o, axis=1).reshape(DH * 16, D)
                    wop_ref[:, pair * 8:(pair + 1) * 8, :] = _pack(z).reshape(DH, 8, D)
            wqkv_copy(j).wait()
            p, pair = j // 2, j % 2
            o = []
            for c in range(2):
                wj = wraw_ref[:, (2 * j + c) * 128:(2 * j + c + 1) * 128]
                o.append(jax.lax.dot_general(perm_q if p == 0 else perm, wj, NT,
                                             preferred_element_type=f32).reshape(DH, 8, D))
            z = jnp.concatenate(o, axis=1).reshape(DH * 16, D)
            wt_ref[p * DH:(p + 1) * DH, pair * 8:(pair + 1) * 8, :] = _pack(z).reshape(DH, 8, D)

    @pl.when(blk < NB - 1)
    def _():
        xf_copy(blk + 1).start()

    xr_copy(blk).wait()

    kv_ref[:, :, 0:HALO, :] = kv_ref[:, :, T:T + HALO, :]

    row128 = jax.lax.broadcasted_iota(jnp.int32, (RC, 128), 0)

    def ln1(l, s):
        for r0 in range(s * TS, (s + 1) * TS, LC):
            xn_ref[r0 // 2:(r0 + LC) // 2, :] = _pack(_ln(xs_ref[r0:r0 + LC, :]))
            yield CLN

    def qkv(l, s):
        for c in range(3 * NC):
            xn = _unpack(xn_ref[hrows(s), :])
            wt = _unpack(wt_ref[4 * c:4 * c + 4].reshape(64, D))
            rc = jax.lax.dot_general(xn, wt, NT, preferred_element_type=f32)
            if c < NC:
                q_ref[c, rows(s), :] = rc * 1.5 if None else rc
            else:
                kv_ref[l, c - NC, HALO + s * TS:HALO + (s + 1) * TS, :] = rc
            yield TS

    def att(l, s):
        for r0 in range(s * TS, (s + 1) * TS, RC):
            q = [q_ref[c, r0:r0 + RC, :] for c in range(NC)]
            ls = []
            for w in range(W):
                b = HALO + r0 - DIL * w
                p = [q[c] * kv_ref[l, c, b:b + RC, :] for c in range(NC)]
                t = (p[0] + p[1]) + (p[2] + p[3])
                t = t + pltpu.roll(t, 64, 1)
                t = t + pltpu.roll(t, 32, 1)
                if r0 < DIL * w:
                    bad = jnp.logical_and(row128 + r0 < DIL * w, blk == 0)
                    t = jnp.where(bad, -1e9, t)
                ls.append(t)
            mx = ls[0]
            for w in range(1, W):
                mx = jnp.maximum(mx, ls[w])
            es = [jnp.exp(x - mx) for x in ls]
            den = es[0]
            for w in range(1, W):
                den = den + es[w]
            inv = 1.0 / den
            outs = []
            for c in range(NC):
                acc = None
                for w in range(W):
                    b = HALO + r0 - DIL * w
                    pv = es[w] * kv_ref[l, NC + c, b:b + RC, :]
                    acc = pv if acc is None else acc + pv
                outs.append(acc * inv)
            a_ref[r0 // 2:(r0 + RC) // 2, :] = _pack(jnp.concatenate(outs, axis=1))
            yield CATT

    def wo(l, s):
        for c in range(NC):
            cs = slice(c * 128, (c + 1) * 128)
            wj = _unpack(wop_ref[:, :, cs].reshape(D // 2, 128))
            xs_ref[rows(s), cs] = xs_ref[rows(s), cs] + jnp.dot(
                _unpack(a_ref[hrows(s), :]), wj, preferred_element_type=f32)
            yield TS

    def ln2(l, s):
        for r0 in range(s * TS, (s + 1) * TS, LC):
            xn_ref[r0 // 2:(r0 + LC) // 2, :] = _pack(_ln(_ln(xs_ref[r0:r0 + LC, :])))
            yield 2 * CLN

    def bias(ref, n0, n1):
        if B1D:
            return ref[n0:n1].astype(f32).reshape(1, n1 - n0)
        return ref[:, n0:n1].astype(f32)

    def w1(l, s):
        for n0 in range(0, F, 128):
            n1 = min(F, n0 + 128)
            y = _unpack(xn_ref[hrows(s), :])
            h = jax.lax.dot_general(y, w1_ref[n0:n1, :], NT, preferred_element_type=f32)
            h = h + bias(b1_ref, n0, n1)
            g_ref[hrows(s), n0:n1] = _pack(_gelu(h))
            yield TS * GW // 100

    def w2(l, s):
        for c in range(NC):
            cs = slice(c * 128, (c + 1) * 128)
            r = xs_ref[rows(s), cs] + jnp.dot(_unpack(g_ref[hrows(s), :]), w2_ref[:, cs],
                                              preferred_element_type=f32) \
                + bias(b2_ref, c * 128, (c + 1) * 128)
            if l == 0:
                xs_ref[rows(s), cs] = r
            else:
                ob_ref[rows(s), cs] = r.astype(bf16)
            yield TS * 11 // 4

    seen = set()
    queue = []
    credit = [0]

    def pump():
        while queue and credit[0] > 0:
            try:
                credit[0] -= next(queue[0][1])
            except StopIteration:
                queue.pop(0)
        if not queue:
            credit[0] = min(credit[0], 0)

    def flush(tag):
        while any(t == tag for t, _ in queue):
            for _ in queue[0][1]:
                pass
            queue.pop(0)

    def run(gen):
        for cost in gen:
            credit[0] += cost
            pump()

    toks = ORDER.split("_")
    for i, tok in enumerate(toks):
        if tok == "W":
            for t in (1, 2, 3):
                if any(tt == t and nm == "ln1_in" for tt, nm in [(a, g.__name__) for a, g in queue]):
                    flush(t)
            @pl.when(blk < NB - 1)
            def _():
                xr_copy(blk + 1).start()

            @pl.when(blk == 0)
            def _():
                b1_copy.wait()
                b2_copy.wait()
                w1_copy.wait()
                w2_copy.wait()

            @pl.when(blk > 0)
            def _():
                o_copy(blk - 1).wait()

            @pl.when(blk < NB - 1)
            def _():
                xf_copy(blk + 1).wait()
            continue
        if tok == "N":
            nxt = pl.multiple_of(jnp.minimum(blk + 1, NB - 1) * T, T)
            queue.append(("N", ln1_in(nxt, 0)))
            continue
        if tok[0] == "L":
            queue.append((int(tok[1]), ln1_in(row0, int(tok[1]))))
            continue
        k, s = tok[0], int(tok[1])
        l = 1 if k.islower() else 0
        k = k.upper()
        assert (k, s, l) not in seen
        seen.add((k, s, l))
        flush(s)
        if k == "Q":
            run(qkv(l, s))
            queue.append((s, att(l, s)))
        elif k == "O":
            run(wo(l, s))
            queue.append((s, ln2(l, s)))
        elif k == "A":
            run(w1(l, s))
        else:
            run(w2(l, s))
            if l == 0:
                queue.append((s, ln1(1, s)))
    flush("N")
    assert len(seen) == 8 * NS and not queue

    o_copy(blk).start()

    @pl.when(blk == NB - 1)
    def _():
        o_copy(blk).wait()


@jax.jit
def pallas_interleave_layers__sliding_local_dilated__mixer_channel_mlp__prompt_kernel(
    A_x, A_wqkv, A_wo, B_x, B_w1, B_b1, B_w2, B_b2):
    x = A_x.reshape(S, D)
    if B1D:
        b1, b2 = B_b1, B_b2
        bspec = lambda n: pl.BlockSpec((n,), lambda i: (0,))
    else:
        b1 = B_b1.reshape(1, F)
        b2 = B_b2.reshape(1, D)
        bspec = lambda n: pl.BlockSpec((1, n), lambda i: (0, 0))
    w1 = B_w1.T
    hbm = pl.BlockSpec(memory_space=pl.ANY)
    out = pl.pallas_call(
        kernel,
        grid=(NB,),
        in_specs=[hbm] * 7,
        out_specs=hbm,
        out_shape=jax.ShapeDtypeStruct((S, D), bf16),
        scratch_shapes=[
            pltpu.VMEM(b1.shape, bf16),
            pltpu.VMEM(b2.shape, bf16),
            pltpu.VMEM((TS, D), bf16),
            pltpu.VMEM((T - TS, D), bf16),
            pltpu.VMEM((T, D), bf16),
            pltpu.VMEM((D, 3 * D), bf16),
            pltpu.VMEM((D, D), bf16),
            pltpu.VMEM((3 * DH, 16, D), u32),
            pltpu.VMEM((DH, 16, D), u32),
            pltpu.VMEM((F, D), bf16),
            pltpu.VMEM((F, D), bf16),
            pltpu.VMEM((T, D), f32),
            pltpu.VMEM((T // 2, D), u32),
            pltpu.VMEM((NC, T, 128), f32),
            pltpu.VMEM((2, 2 * NC, HALO + T, 128), f32),
            pltpu.VMEM((T // 2, D), u32),
            pltpu.VMEM((T // 2, F), u32),
            pltpu.SemaphoreType.DMA((14,)),
        ],
        compiler_params=pltpu.CompilerParams(
            dimension_semantics=("arbitrary",),
            vmem_limit_bytes=64 * 1024 * 1024,
        ),
    )(x, A_wqkv, A_wo, w1, b1, B_w2, b2)
    return out.reshape(1, S, D)
```

```python
import functools
import jax
import jax.numpy as jnp
import jax.experimental.pallas as pl
import jax.experimental.pallas.tpu as pltpu

S, D, F = 2048, 512, 1376
H, DH, W, DIL = 32, 16, 8, 2
T = int("512")
TS = int("128")
RC = int("16")
LC = int("32")
CATT = int("160")
CLN = int("100")
GW = int("50")
ORDER = 'Q0_L1_Q1_L2_O0_L3_Q2_O1_W_A0_Q3_O2_A1_A2_B0_O3_B1_q0_A3_B2_q1_o0_q2_B3_o1_a0_q3_a1_o2_b1_a2_b0_N_o3_b2_a3_b3'
DEPD = int("0")
DEPV = "out"
QORD = "qkv"
TIE = int("0")
TIEL = int("0")
NOATT = "B"
MD = int("0")
MB = int("1")
PACKW = int("3")
EXP2 = int("1")
RCP = int("1")
GEL = int("1")
STAGE = int("10")
B1D = int("1")
NS = T // TS
NB = S // T
HALO = 16
EPS = 1e-5
NC = D // 128
f32 = jnp.float32
bf16 = jnp.bfloat16
u32 = jnp.uint32
NT = (((1,), (1,)), ((), ()))
LOG2E = 1.4426950408889634


def _ln(x):
    m = jnp.mean(x, axis=-1, keepdims=True)
    xc = x - m
    v = jnp.mean(xc * xc, axis=-1, keepdims=True)
    return xc * jax.lax.rsqrt(v + EPS)


def _gelu(x):
    c = 0.7978845608028654
    if GEL:
        hx = 0.5 * x
        return hx + hx * jnp.tanh(x * (c + (c * 0.044715) * (x * x)))
    return 0.5 * x * (1.0 + jnp.tanh(c * (x + 0.044715 * (x * x * x))))


def _pack(x):
    return pltpu.bitcast(x.astype(bf16), u32)


def _unpack(x):
    return pltpu.bitcast(x, bf16)


def kernel(x_hbm, wqkv_hbm, wo_hbm, w1_hbm, b1_hbm, w2_hbm, b2_hbm, o_hbm,
           b1_ref, b2_ref, xf_ref, xr_ref, ob_ref, wraw_ref, woraw_ref, wt_ref, wop_ref, w1_ref, w2_ref, w1p_ref, w2p_ref,
           xs_ref, xn_ref, q_ref, kv_ref, a_ref, g_ref, z_ref, t_ref, l_ref, u_ref, e_ref, st_ref,
           sem_w):
    blk = pl.program_id(0)
    row0 = pl.multiple_of(blk * T, T)

    def xf_copy(b):
        return pltpu.make_async_copy(x_hbm.at[pl.ds(b * T, TS), :], xf_ref, sem_w.at[9])

    def xr_copy(b):
        return pltpu.make_async_copy(x_hbm.at[pl.ds(b * T + TS, T - TS), :], xr_ref,
                                     sem_w.at[10])

    def o_copy(b):
        return pltpu.make_async_copy(ob_ref.at[pl.ds(0, T - TS), :], o_hbm.at[pl.ds(b * T, T - TS), :],
                                     sem_w.at[11])

    def o2_copy(b):
        return pltpu.make_async_copy(ob_ref.at[pl.ds(T - TS, TS), :],
                                     o_hbm.at[pl.ds(b * T + T - TS, TS), :], sem_w.at[14])

    def wqkv_copy(j):
        return pltpu.make_async_copy(wqkv_hbm.at[:, pl.ds(j * 256, 256)], wraw_ref.at[:, pl.ds(j * 256, 256)],
                                     sem_w.at[j])

    wo_copy = pltpu.make_async_copy(wo_hbm, woraw_ref, sem_w.at[6])
    w1_copy = pltpu.make_async_copy(w1_hbm, w1_ref, sem_w.at[7])
    w2_copy = pltpu.make_async_copy(w2_hbm, w2_ref, sem_w.at[8])
    b1_copy = pltpu.make_async_copy(b1_hbm, b1_ref, sem_w.at[12])
    b2_copy = pltpu.make_async_copy(b2_hbm, b2_ref, sem_w.at[13])

    last = [None]

    def tie(xs_):
        if last[0] is None:
            return xs_
        dep = pltpu.bitcast(last[0], jnp.int32) & z_ref[...]
        return [pltpu.bitcast(pltpu.bitcast(x, jnp.int32) | dep, f32) for x in xs_]

    def tie_wide(x):
        if last[0] is None or not TIEL:
            return x
        dep = pltpu.bitcast(last[0], jnp.int32) & z_ref[...]
        dep = jnp.concatenate([jnp.concatenate([dep] * (LC // RC), axis=0)] * NC, axis=1)
        return pltpu.bitcast(pltpu.bitcast(x, jnp.int32) | dep, f32)

    tiles = []

    def chain(lhs):
        if MD == 0 or len(tiles) < MD:
            return lhs
        dep = pltpu.bitcast(tiles[-MD], u32) & pltpu.bitcast(z_ref[0:8, :], u32)
        k = lhs.shape[1]
        head = lhs[0:8, 0:D] | jnp.concatenate([dep] * NC, axis=1)
        if k > D:
            head = jnp.concatenate([head, lhs[0:8, D:]], axis=1)
        return jnp.concatenate([head, lhs[8:]], axis=0)

    def rows(s):
        return slice(s * TS, (s + 1) * TS)

    def hrows(s):
        return slice(s * TS // 2, (s + 1) * TS // 2)

    def ln_ref(r0, twice):
        rs = slice(r0, r0 + LC)
        wide = lambda v: jnp.concatenate([v] * NC, axis=1)
        m = jnp.mean(xs_ref[rs, :], axis=-1, keepdims=True)
        st_ref[0, rs, :] = jnp.broadcast_to(m, (LC, 128))
        xc = xs_ref[rs, :] - wide(st_ref[0, rs, :])
        v = jnp.mean(xc * xc, axis=-1, keepdims=True)
        st_ref[1, rs, :] = jnp.broadcast_to(jax.lax.rsqrt(v + EPS), (LC, 128))
        y = (xs_ref[rs, :] - wide(st_ref[0, rs, :])) * wide(st_ref[1, rs, :])
        if not twice:
            return y
        m2 = jnp.mean(y, axis=-1, keepdims=True)
        st_ref[2, rs, :] = jnp.broadcast_to(m2, (LC, 128))
        yc = (xs_ref[rs, :] - wide(st_ref[0, rs, :])) * wide(st_ref[1, rs, :]) - wide(st_ref[2, rs, :])
        v2 = jnp.mean(yc * yc, axis=-1, keepdims=True)
        st_ref[3, rs, :] = jnp.broadcast_to(jax.lax.rsqrt(v2 + EPS), (LC, 128))
        return ((xs_ref[rs, :] - wide(st_ref[0, rs, :])) * wide(st_ref[1, rs, :])
                - wide(st_ref[2, rs, :])) * wide(st_ref[3, rs, :])

    def ln1_in(base, s):
        for r0 in range(s * TS, (s + 1) * TS, LC):
            x = (xf_ref[r0:r0 + LC, :] if s == 0 else xr_ref[r0 - TS:r0 - TS + LC, :]).astype(f32)
            xs_ref[r0:r0 + LC, :] = x
            xn_ref[r0 // 2:(r0 + LC) // 2, :] = _pack(ln_ref(r0, False) if STAGE & 32 else _ln(x))
            yield CLN

    @pl.when(blk == 0)
    def _():
        xf_copy(0).start()
        for j in range(4):
            wqkv_copy(j).start()
        wo_copy.start()
        for j in range(4, 6):
            wqkv_copy(j).start()
        xr_copy(0).start()
        b1_copy.start()
        b2_copy.start()
        w1_copy.start()
        w2_copy.start()
        kv_ref[:, :, T:T + HALO, :] = jnp.zeros((2, 2 * NC, HALO, 128), f32)
        z_ref[...] = jnp.zeros(z_ref.shape, jnp.int32)
        rho = jax.lax.broadcasted_iota(jnp.int32, (128, 128), 0)
        col = jax.lax.broadcasted_iota(jnp.int32, (128, 128), 1)
        hit = rho == (col % DH) * 8 + col // DH
        perm = jnp.where(hit, 1.0, 0.0).astype(bf16)
        perm_q = jnp.where(hit, DH ** -0.5, 0.0).astype(bf16)
        xf_copy(0).wait()
        list(ln1_in(0, 0))
        for j in range(6):
            if j == 4:
                wo_copy.wait()
                for pair in range(2):
                    o = []
                    for c in range(2):
                        wj = woraw_ref[(2 * pair + c) * 128:(2 * pair + c + 1) * 128, :]
                        o.append(jnp.dot(perm, wj, preferred_element_type=f32).reshape(DH, 8, D))
                    z = jnp.concatenate(o, axis=1).reshape(DH * 16, D)
                    wop_ref[:, pair * 8:(pair + 1) * 8, :] = _pack(z).reshape(DH, 8, D)
            wqkv_copy(j).wait()
            p, pair = j // 2, j % 2
            o = []
            for c in range(2):
                wj = wraw_ref[:, (2 * j + c) * 128:(2 * j + c + 1) * 128]
                o.append(jax.lax.dot_general(perm_q if p == 0 else perm, wj, NT,
                                             preferred_element_type=f32).reshape(DH, 8, D))
            z = jnp.concatenate(o, axis=1).reshape(DH * 16, D)
            wt_ref[p * DH:(p + 1) * DH, pair * 8:(pair + 1) * 8, :] = _pack(z).reshape(DH, 8, D)

    @pl.when(blk < NB - 1)
    def _():
        xf_copy(blk + 1).start()

    xr_copy(blk).wait()

    kv_ref[:, :, 0:HALO, :] = kv_ref[:, :, T:T + HALO, :]

    row128 = jax.lax.broadcasted_iota(jnp.int32, (RC, 128), 0)

    def ln1(l, s):
        for r0 in range(s * TS, (s + 1) * TS, LC):
            xn_ref[r0 // 2:(r0 + LC) // 2, :] = _pack(ln_ref(r0, False) if STAGE & 32 else _ln(xs_ref[r0:r0 + LC, :]))
            yield CLN

    def qkv(l, s):
        for c in [4 * "qkv".index(ch) + i for ch in QORD for i in range(NC)]:
            xn = _unpack(chain(xn_ref[hrows(s), :]))
            wt = _unpack(wt_ref[4 * c:4 * c + 4].reshape(64, D))
            rc = jax.lax.dot_general(xn, wt, NT, preferred_element_type=f32)
            last[0] = rc[TS - RC:, :]
            tiles.append(rc[TS - 8:, :])
            if c < NC:
                q_ref[c, rows(s), :] = rc * LOG2E if EXP2 else rc
            else:
                kv_ref[l, c - NC, HALO + s * TS:HALO + (s + 1) * TS, :] = rc
            yield TS

    hist = []

    def att(l, s):
        del hist[:]
        for r0 in range(s * TS, (s + 1) * TS, RC):
            q = [q_ref[c, r0:r0 + RC, :] for c in range(NC)]
            if TIE:
                q = tie(q)
            if DEPD > 0 and len(hist) >= DEPD:
                dep = pltpu.bitcast(hist[-DEPD], jnp.int32) & z_ref[...]
                q = [pltpu.bitcast(pltpu.bitcast(x, jnp.int32) | dep, f32) for x in q]
            ls = []
            for w in range(W):
                b = HALO + r0 - DIL * w
                p = [q[c] * kv_ref[l, c, b:b + RC, :] for c in range(NC)]
                t = (p[0] + p[1]) + (p[2] + p[3])
                if STAGE & 1:
                    t_ref[w, r0:r0 + RC, :] = t
                    t = t_ref[w, r0:r0 + RC, :]
                rr = pltpu.roll(t, 64, 1)
                if STAGE & 4:
                    t_ref[w, r0:r0 + RC, :] = t
                    t = t_ref[w, r0:r0 + RC, :]
                t = t + rr
                rr = pltpu.roll(t, 32, 1)
                if STAGE & 8:
                    u_ref[w, r0:r0 + RC, :] = t
                    t = u_ref[w, r0:r0 + RC, :]
                t = t + rr
                if r0 < DIL * w:
                    bad = jnp.logical_and(row128 + r0 < DIL * w, blk == 0)
                    t = jnp.where(bad, -1e9, t)
                if STAGE & 2:
                    l_ref[w, r0:r0 + RC, :] = t
                    t = l_ref[w, r0:r0 + RC, :]
                ls.append(t)
            mx = ls[0]
            for w in range(1, W):
                mx = jnp.maximum(mx, ls[w])
            es = [(jnp.exp2 if EXP2 else jnp.exp)(x - mx) for x in ls]
            den = es[0]
            for w in range(1, W):
                den = den + es[w]
            if RCP:
                inv = pl.reciprocal(den, approx=True)
                inv = inv * (2.0 - den * inv)
            else:
                inv = 1.0 / den
            outs = []
            if STAGE & 16:
                for w in range(W):
                    e_ref[w, r0:r0 + RC, :] = es[w]
                es = [e_ref[w, r0:r0 + RC, :] for w in range(W)]
            for c in range(NC):
                acc = None
                for w in range(W):
                    b = HALO + r0 - DIL * w
                    pv = es[w] * kv_ref[l, NC + c, b:b + RC, :]
                    acc = pv if acc is None else acc + pv
                outs.append(acc * inv)
            hist.append({"mx": mx, "den": den, "inv": inv, "out": outs[NC - 1],
                         "outs": (outs[0] + outs[1]) + (outs[2] + outs[3])}[DEPV])
            a_ref[r0 // 2:(r0 + RC) // 2, :] = _pack(jnp.concatenate(outs, axis=1))
            yield CATT

    def wo(l, s):
        for c in range(NC):
            cs = slice(c * 128, (c + 1) * 128)
            wj = _unpack(wop_ref[:, :, cs].reshape(D // 2, 128))
            r = jnp.dot(_unpack(chain(a_ref[hrows(s), :])), wj, preferred_element_type=f32)
            last[0] = r[TS - RC:, :]
            tiles.append(r[TS - 8:, :])
            xs_ref[rows(s), cs] = xs_ref[rows(s), cs] + r
            yield TS

    def ln2(l, s):
        for r0 in range(s * TS, (s + 1) * TS, LC):
            xn_ref[r0 // 2:(r0 + LC) // 2, :] = _pack(ln_ref(r0, True) if STAGE & 32 else _ln(_ln(xs_ref[r0:r0 + LC, :])))
            yield 2 * CLN

    def bias(ref, n0, n1):
        if B1D:
            return ref[n0:n1].astype(f32).reshape(1, n1 - n0)
        return ref[:, n0:n1].astype(f32)

    def w1(l, s, first):
        for n0 in range(0, F, 128):
            n1 = min(F, n0 + 128)
            y = _unpack(chain(xn_ref[hrows(s), :]))
            if not PACKW & 1:
                wj = w1_ref[n0:n1, :]
            elif first:
                wj = w1_ref[n0:n1, :]
                w1p_ref[n0 // 2:n1 // 2, :] = pltpu.bitcast(wj, u32)
            else:
                wj = _unpack(w1p_ref[n0 // 2:n1 // 2, :])
            h = jax.lax.dot_general(y, wj, NT, preferred_element_type=f32)
            if n1 - n0 == 128:
                last[0] = h[TS - RC:, :]
                tiles.append(h[TS - 8:, :])
            h = h + bias(b1_ref, n0, n1)
            g_ref[hrows(s), n0:n1] = _pack(_gelu(h))
            yield TS * GW // 100

    def w2(l, s, first):
        for c in range(NC):
            cs = slice(c * 128, (c + 1) * 128)
            if not PACKW & 2:
                wj = w2_ref[:, cs]
            elif first:
                wj = w2_ref[:, cs]
                w2p_ref[:, cs] = pltpu.bitcast(wj, u32)
            else:
                wj = _unpack(w2p_ref[:, cs])
            r = xs_ref[rows(s), cs] + jnp.dot(_unpack(chain(g_ref[hrows(s), :])), wj,
                                              preferred_element_type=f32) \
                + bias(b2_ref, c * 128, (c + 1) * 128)
            last[0] = r[TS - RC:, :]
            tiles.extend([r[TS - 8:, :]] * MB)
            if l == 0:
                xs_ref[rows(s), cs] = r
            else:
                ob_ref[rows(s), cs] = r.astype(bf16)
            yield TS * 11 // 4

    seen = set()
    queue = []
    credit = [0]

    def pump(kind):
        while credit[0] > 0:
            cand = [e for e in queue if not (e[1].__name__ == "att" and kind in NOATT)]
            if not cand:
                break
            try:
                credit[0] -= next(cand[0][1])
            except StopIteration:
                queue.remove(cand[0])
        credit[0] = min(credit[0], 0)

    def flush(tag):
        for e in [e for e in queue if e[0] == tag]:
            for _ in e[1]:
                pass
            queue.remove(e)

    def run(gen, kind):
        for cost in gen:
            credit[0] += cost
            pump(kind)

    toks = ORDER.split("_")
    for i, tok in enumerate(toks):
        if tok == "W":
            last[0] = None
            del tiles[:]
            for t in range(1, NS):
                if any(tt == t and nm == "ln1_in" for tt, nm in [(a, g.__name__) for a, g in queue]):
                    flush(t)
            @pl.when(blk < NB - 1)
            def _():
                xr_copy(blk + 1).start()

            @pl.when(blk == 0)
            def _():
                b1_copy.wait()
                b2_copy.wait()
                w1_copy.wait()
                w2_copy.wait()

            @pl.when(blk > 0)
            def _():
                o_copy(blk - 1).wait()
                o2_copy(blk - 1).wait()

            @pl.when(blk < NB - 1)
            def _():
                xf_copy(blk + 1).wait()
            continue
        if tok == "N":
            nxt = pl.multiple_of(jnp.minimum(blk + 1, NB - 1) * T, T)
            queue.append(("N", ln1_in(nxt, 0)))
            continue
        if tok[0] == "L":
            queue.append((int(tok[1]), ln1_in(row0, int(tok[1]))))
            continue
        k, s = tok[0], int(tok[1])
        l = 1 if k.islower() else 0
        k = k.upper()
        assert (k, s, l) not in seen
        seen.add((k, s, l))
        flush(s)
        if tok == "b" + str(NS - 1):
            assert i == len(toks) - 1
            o_copy(blk).start()
        if k == "Q":
            run(qkv(l, s), k)
            queue.append((s, att(l, s)))
        elif k == "O":
            run(wo(l, s), k)
            queue.append((s, ln2(l, s)))
        elif k == "A":
            run(w1(l, s, sum(e[0] == 'A' for e in seen) == 1), k)
        else:
            run(w2(l, s, sum(e[0] == 'B' for e in seen) == 1), k)
            if l == 0:
                queue.append((s, ln1(1, s)))
    flush("N")
    assert len(seen) == 8 * NS and not queue

    o2_copy(blk).start()

    @pl.when(blk == NB - 1)
    def _():
        o_copy(blk).wait()
        o2_copy(blk).wait()


@jax.jit
def pallas_interleave_layers__sliding_local_dilated__mixer_channel_mlp__prompt_kernel(
    A_x, A_wqkv, A_wo, B_x, B_w1, B_b1, B_w2, B_b2):
    x = A_x.reshape(S, D)
    if B1D:
        b1, b2 = B_b1, B_b2
        bspec = lambda n: pl.BlockSpec((n,), lambda i: (0,))
    else:
        b1 = B_b1.reshape(1, F)
        b2 = B_b2.reshape(1, D)
        bspec = lambda n: pl.BlockSpec((1, n), lambda i: (0, 0))
    w1 = B_w1.T
    hbm = pl.BlockSpec(memory_space=pl.ANY)
    out = pl.pallas_call(
        kernel,
        grid=(NB,),
        in_specs=[hbm] * 7,
        out_specs=hbm,
        out_shape=jax.ShapeDtypeStruct((S, D), bf16),
        scratch_shapes=[
            pltpu.VMEM(b1.shape, bf16),
            pltpu.VMEM(b2.shape, bf16),
            pltpu.VMEM((TS, D), bf16),
            pltpu.VMEM((T - TS, D), bf16),
            pltpu.VMEM((T, D), bf16),
            pltpu.VMEM((D, 3 * D), bf16),
            pltpu.VMEM((D, D), bf16),
            pltpu.VMEM((3 * DH, 16, D), u32),
            pltpu.VMEM((DH, 16, D), u32),
            pltpu.VMEM((F, D), bf16),
            pltpu.VMEM((F, D), bf16),
            pltpu.VMEM((F // 2, D), u32),
            pltpu.VMEM((F // 2, D), u32),
            pltpu.VMEM((T, D), f32),
            pltpu.VMEM((T // 2, D), u32),
            pltpu.VMEM((NC, T, 128), f32),
            pltpu.VMEM((2, 2 * NC, HALO + T, 128), f32),
            pltpu.VMEM((T // 2, D), u32),
            pltpu.VMEM((T // 2, F), u32),
            pltpu.VMEM((RC, 128), jnp.int32),
            pltpu.VMEM((W, T, 128), f32),
            pltpu.VMEM((W, T, 128), f32),
            pltpu.VMEM((W, T, 128), f32),
            pltpu.VMEM((W, T, 128), f32),
            pltpu.VMEM((4, T, 128), f32),
            pltpu.SemaphoreType.DMA((15,)),
        ],
        compiler_params=pltpu.CompilerParams(
            dimension_semantics=("arbitrary",),
            vmem_limit_bytes=64 * 1024 * 1024,
        ),
    )(x, A_wqkv, A_wo, w1, b1, B_w2, b2)
    return out.reshape(1, S, D)
```

```python
import jax
import jax.numpy as jnp
import jax.experimental.pallas as pl
import jax.experimental.pallas.tpu as pltpu

S, D, F = 2048, 512, 1376
H, DH, W, DIL = 32, 16, 8, 2
T = 512
TS = 128
RC = 16
LC = 32
NS = T // TS
NB = S // T
HALO = 16
EPS = 1e-5
NC = D // 128
f32 = jnp.float32
bf16 = jnp.bfloat16
u32 = jnp.uint32
NN = (((1,), (0,)), ((), ()))
NT = (((1,), (1,)), ((), ()))
LOG2E = 1.4426950408889634

ORDER = ("L1_Q0_Q1_L2_O0_Q2_O1_L3_Q3_O2_W_A1_A0_B1_B0_A2_O3_B2_q0_q1_q2_o0_A3_B3_a0_o1_q3_"
         "a1_o2_b1_b0_a2_o3_b2_N_a3_b3")
PRO = ("wq0_Pq0_wq1_X0_Pq1_Q0q_X1_wk_Pk_L1_Q1q_Q0k_wv_Pv_Q1k_Q1v_Q0v_t06_X2_wo_L2_t1_L3_Po_"
       "t0_Q2_O0_n0_O1_t2_n1_Q3_O2_t3")
CATT = 160
CLN = 100


def _ln(x):
    m = jnp.mean(x, axis=-1, keepdims=True)
    xc = x - m
    v = jnp.mean(xc * xc, axis=-1, keepdims=True)
    return xc * jax.lax.rsqrt(v + EPS)


def _gelu(x):
    c = 0.7978845608028654
    hx = 0.5 * x
    return hx + hx * jnp.tanh(x * (c + (c * 0.044715) * (x * x)))


def _pack(x):
    return pltpu.bitcast(x.astype(bf16), u32)


def _unpack(x):
    return pltpu.bitcast(x, bf16)


def _plan():
    tiles = {"Q": [TS] * (3 * NC), "O": [TS] * NC, "A": [TS // 2] * (-(-F // 128)),
             "B": [TS * 11 // 4] * NC}
    chunks = {"att": [CATT] * (TS // RC), "ln1": [CLN] * (TS // LC),
              "ln2": [2 * CLN] * (TS // LC), "lnx": [CLN] * (TS // LC)}
    plans = [[], []]
    cur = plans[0]
    queue = []
    credit = 0
    seen = []

    def emit(e):
        cur.append((e[1], e[2], e[3], e[4], False))
        e[4] += 1
        if e[4] == len(chunks[e[1]]):
            queue.remove(e)

    def flush(pred):
        for e in [e for e in queue if pred(e)]:
            while e in queue:
                emit(e)

    for tok in ORDER.split("_"):
        if tok == "W":
            flush(lambda e: e[1] == "lnx")
            cur = plans[1]
            continue
        if tok == "N":
            queue.append(["N", "lnx", 0, 0, 0])
            continue
        k, s = tok[0], int(tok[1])
        if k == "L":
            queue.append([s, "lnx", 0, s, 0])
            continue
        l = 1 if k.islower() else 0
        k = k.upper()
        first = all(e[0] != k for e in seen)
        seen.append((k, l, s))
        flush(lambda e: e[0] == s)
        for i, cost in enumerate(tiles[k]):
            cur.append((k, l, s, i, first))
            credit += cost
            while credit > 0:
                cand = [e for e in queue if not (e[1] == "att" and k == "B")]
                if not cand:
                    break
                credit -= chunks[cand[0][1]][0]
                emit(cand[0])
            credit = min(credit, 0)
        if k == "Q":
            queue.append([s, "att", l, s, 0])
        elif k == "O":
            queue.append([s, "ln2", l, s, 0])
        elif k == "B" and l == 0:
            queue.append([s, "ln1", 1, s, 0])
    flush(lambda e: True)
    assert len(set(seen)) == 8 * NS
    return plans


def _kernel(x_hbm, wqkv_hbm, wo_hbm, w1_hbm, b1_hbm, w2_hbm, b2_hbm, o_hbm,
            b1_ref, b2_ref, xf_ref, xr_ref, ob_ref, wraw_ref, woraw_ref, wt_ref, wop_ref,
            w1_ref, w2_ref, w1p_ref, w2p_ref,
            xs_ref, xn_ref, q_ref, kv_ref, a_ref, g_ref, l_ref, u_ref, sem):
    blk = pl.program_id(0)

    def xf_copy(b):
        return pltpu.make_async_copy(x_hbm.at[pl.ds(b * T, TS), :], xf_ref, sem.at[0])

    def xr_copy(b):
        return pltpu.make_async_copy(x_hbm.at[pl.ds(b * T + TS, T - TS), :], xr_ref, sem.at[1])

    x1_copy = pltpu.make_async_copy(x_hbm.at[pl.ds(TS, TS), :], xr_ref.at[pl.ds(0, TS), :], sem.at[1])
    x2_copy = pltpu.make_async_copy(x_hbm.at[pl.ds(2 * TS, T - 2 * TS), :],
                                    xr_ref.at[pl.ds(TS, T - 2 * TS), :], sem.at[2])

    def o_copy(b):
        return pltpu.make_async_copy(ob_ref.at[pl.ds(0, T - TS), :], o_hbm.at[pl.ds(b * T, T - TS), :],
                                     sem.at[2])

    def o2_copy(b):
        return pltpu.make_async_copy(ob_ref.at[pl.ds(T - TS, TS), :],
                                     o_hbm.at[pl.ds(b * T + T - TS, TS), :], sem.at[3])

    def wqkv_copy(p, half=None):
        if half is None:
            return pltpu.make_async_copy(wqkv_hbm.at[:, pl.ds(p * D, D)], wraw_ref.at[:, pl.ds(p * D, D)],
                                         sem.at[4 + p])
        c0 = p * D + half * (D // 2)
        return pltpu.make_async_copy(wqkv_hbm.at[:, pl.ds(c0, D // 2)], wraw_ref.at[:, pl.ds(c0, D // 2)],
                                     sem.at[4 + p if half == 0 else 3])

    wo_copy = pltpu.make_async_copy(wo_hbm, woraw_ref, sem.at[7])
    late_copies = [pltpu.make_async_copy(src, dst, sem.at[8]) for src, dst in (
        (b1_hbm, b1_ref), (b2_hbm, b2_ref), (w1_hbm, w1_ref), (w2_hbm, w2_ref))]

    def rows(s):
        return slice(s * TS, (s + 1) * TS)

    def hrows(s):
        return slice(s * TS // 2, (s + 1) * TS // 2)

    row128 = jax.lax.broadcasted_iota(jnp.int32, (RC, 128), 0)

    def lnx(l, s, i, first, first_block):
        r0 = s * TS + i * LC
        x = (xf_ref[r0:r0 + LC, :] if s == 0 else xr_ref[r0 - TS:r0 - TS + LC, :]).astype(f32)
        xs_ref[r0:r0 + LC, :] = x
        xn_ref[r0 // 2:(r0 + LC) // 2, :] = _pack(_ln(x))

    def ln1(l, s, i, first, first_block):
        r0 = s * TS + i * LC
        xn_ref[r0 // 2:(r0 + LC) // 2, :] = _pack(_ln(xs_ref[r0:r0 + LC, :]))

    def ln2(l, s, i, first, first_block):
        r0 = s * TS + i * LC
        xn_ref[r0 // 2:(r0 + LC) // 2, :] = _pack(_ln(_ln(xs_ref[r0:r0 + LC, :])))

    def qkv(l, s, c, first, first_block):
        xn = _unpack(xn_ref[hrows(s), :])
        wt = _unpack(wt_ref[4 * c:4 * c + 4].reshape(64, D))
        rc = jax.lax.dot_general(xn, wt, NT, preferred_element_type=f32)
        if c < NC:
            q_ref[c, rows(s), :] = rc * LOG2E
        else:
            kv_ref[l, c - NC, HALO + s * TS:HALO + (s + 1) * TS, :] = rc

    def att(l, s, i, first, first_block):
        r0 = s * TS + i * RC
        q = [q_ref[c, r0:r0 + RC, :] for c in range(NC)]
        ls = []
        for w in range(W):
            b = HALO + r0 - DIL * w
            p = [q[c] * kv_ref[l, c, b:b + RC, :] for c in range(NC)]
            t = (p[0] + p[1]) + (p[2] + p[3])
            t = t + pltpu.roll(t, 64, 1)
            rr = pltpu.roll(t, 32, 1)
            u_ref[w, r0:r0 + RC, :] = t
            t = u_ref[w, r0:r0 + RC, :] + rr
            if r0 < DIL * w and first_block is not False:
                bad = row128 + r0 < DIL * w
                if first_block is not True:
                    bad = jnp.logical_and(bad, first_block)
                t = jnp.where(bad, -1e9, t)
            l_ref[w, r0:r0 + RC, :] = t
            ls.append(l_ref[w, r0:r0 + RC, :])
        mx = ls[0]
        for w in range(1, W):
            mx = jnp.maximum(mx, ls[w])
        es = [jnp.exp2(x - mx) for x in ls]
        den = es[0]
        for w in range(1, W):
            den = den + es[w]
        inv = pl.reciprocal(den, approx=True)
        inv = inv * (2.0 - den * inv)
        outs = []
        for c in range(NC):
            acc = None
            for w in range(W):
                b = HALO + r0 - DIL * w
                pv = es[w] * kv_ref[l, NC + c, b:b + RC, :]
                acc = pv if acc is None else acc + pv
            outs.append(acc * inv)
        a_ref[r0 // 2:(r0 + RC) // 2, :] = _pack(jnp.concatenate(outs, axis=1))

    def wo(l, s, c, first, first_block):
        cs = slice(c * 128, (c + 1) * 128)
        wj = _unpack(wop_ref[:, :, cs].reshape(D // 2, 128))
        r = jnp.dot(_unpack(a_ref[hrows(s), :]), wj, preferred_element_type=f32)
        xs_ref[rows(s), cs] = xs_ref[rows(s), cs] + r

    def bias(ref, n0, n1):
        return ref[n0:n1].astype(f32).reshape(1, n1 - n0)

    def w1(l, s, i, first, first_block):
        n0 = i * 128
        n1 = min(F, n0 + 128)
        y = _unpack(xn_ref[hrows(s), :])
        if first:
            wj = w1_ref[n0:n1, :]
            w1p_ref[n0 // 2:n1 // 2, :] = pltpu.bitcast(wj, u32)
        else:
            wj = _unpack(w1p_ref[n0 // 2:n1 // 2, :])
        if n1 - n0 < 128:
            h = jax.lax.dot_general(wj, y, NT, preferred_element_type=f32).T
        else:
            h = jax.lax.dot_general(y, wj, NT, preferred_element_type=f32)
        h = h + bias(b1_ref, n0, n1)
        g_ref[hrows(s), n0:n1] = _pack(_gelu(h))

    def w2(l, s, c, first, first_block):
        cs = slice(c * 128, (c + 1) * 128)
        if l == 1 and s == NS - 1 and c == 0:
            o_copy(blk).start()
        if first:
            wj = w2_ref[:, cs]
            w2p_ref[:, cs] = pltpu.bitcast(wj, u32)
        else:
            wj = _unpack(w2p_ref[:, cs])
        r = xs_ref[rows(s), cs] + jnp.dot(_unpack(g_ref[hrows(s), :]), wj, preferred_element_type=f32) \
            + bias(b2_ref, c * 128, (c + 1) * 128)
        if l == 0:
            xs_ref[rows(s), cs] = r
        else:
            ob_ref[rows(s), cs] = r.astype(bf16)

    fns = {"Q": qkv, "O": wo, "A": w1, "B": w2, "att": att, "ln1": ln1, "ln2": ln2, "lnx": lnx}

    def run(items, first_block):
        for kind, l, s, i, first in items:
            fns[kind](l, s, i, first, first_block)

    plan1, plan2 = _plan()

    @pl.when(blk == 0)
    def _():
        wqkv_copy(0, 0).start()
        xf_copy(0).start()
        wqkv_copy(0, 1).start()
        x1_copy.start()
        wqkv_copy(1).start()
        wqkv_copy(2).start()
        x2_copy.start()
        wo_copy.start()
        for cp in late_copies:
            cp.start()
        kv_ref[:, :, 0:HALO, :] = jnp.zeros((2, 2 * NC, HALO, 128), f32)
        rho = jax.lax.broadcasted_iota(jnp.int32, (128, 128), 0)
        col = jax.lax.broadcasted_iota(jnp.int32, (128, 128), 1)
        hit = rho == (col % DH) * 8 + col // DH

        def permute(dst, p, scale, get, dims, pairs=(0, 1)):
            perm = jnp.where(hit, scale, 0.0).astype(bf16)
            for pair in pairs:
                o = [jax.lax.dot_general(perm, get(2 * pair + c), dims,
                                         preferred_element_type=f32).reshape(DH, 8, D) for c in range(2)]
                z = jnp.concatenate(o, axis=1).reshape(DH * 16, D)
                dst[p * DH:(p + 1) * DH, pair * 8:(pair + 1) * 8, :] = _pack(z).reshape(DH, 8, D)

        left = list(plan1)

        def take(tok):
            k, s = tok[0], int(tok[1])
            kind = {"t": "att", "n": "ln2", "L": "lnx"}.get(k, k)
            sel = [e for e in left if e[0] == kind and e[2] == s]
            if len(tok) > 2:
                if kind == "Q":
                    sel = [e for e in sel if e[3] // NC == "qkv".index(tok[2])]
                else:
                    sel = sel[:int(tok[2:])]
            for e in sel:
                left.remove(e)
            run(sel, True)

        for tok in PRO.split("_"):
            if tok[0] == "P" and tok[1] in "qkv":
                p = "qkv".index(tok[1])
                half = int(tok[2]) if len(tok) > 2 else None
                permute(wt_ref, p, DH ** -0.5 if p == 0 else 1.0,
                        lambda c: wraw_ref[:, (p * NC + c) * 128:(p * NC + c + 1) * 128], NT,
                        (0, 1) if half is None else (half,))
            elif tok[0] == "w" and tok[1] in "qkv":
                wqkv_copy("qkv".index(tok[1]), int(tok[2]) if len(tok) > 2 else None).wait()
            elif tok == "wo":
                wo_copy.wait()
            elif tok == "X0":
                xf_copy(0).wait()
                run([("lnx", 0, 0, i, False) for i in range(TS // LC)], True)
            elif tok == "Po":
                permute(wop_ref, 0, 1.0, lambda c: woraw_ref[c * 128:(c + 1) * 128, :], NN)
            elif tok == "X1":
                xf_copy(1).start()
                x1_copy.wait()
            elif tok == "X2":
                x2_copy.wait()
            else:
                take(tok)
        assert not left

    @pl.when(blk < NB - 1)
    def _():
        xr_copy(blk + 1).start()

    @pl.when(blk == 0)
    def _():
        for cp in late_copies:
            cp.wait()

    @pl.when(blk > 0)
    def _():
        o_copy(blk - 1).wait()
        o2_copy(blk - 1).wait()

    @pl.when(blk < NB - 1)
    def _():
        xf_copy(blk + 1).wait()

    run(plan2, blk == 0)

    o2_copy(blk).start()

    @pl.when(blk < NB - 2)
    def _():
        xf_copy(blk + 2).start()

    @pl.when(blk < NB - 1)
    def _():
        xr_copy(blk + 1).wait()
        kv_ref[:, :, 0:HALO, :] = kv_ref[:, :, T:T + HALO, :]
        run(plan1, False)

    @pl.when(blk == NB - 1)
    def _():
        o_copy(blk).wait()
        o2_copy(blk).wait()


@jax.jit
def pallas_interleave_layers__sliding_local_dilated__mixer_channel_mlp__prompt_kernel(
    A_x: jax.Array,
    A_wqkv: jax.Array,
    A_wo: jax.Array,
    B_x: jax.Array,
    B_w1: jax.Array,
    B_b1: jax.Array,
    B_w2: jax.Array,
    B_b2: jax.Array,
):
    hbm = pl.BlockSpec(memory_space=pl.ANY)
    out = pl.pallas_call(
        _kernel,
        grid=(NB,),
        in_specs=[hbm] * 7,
        out_specs=hbm,
        out_shape=jax.ShapeDtypeStruct((S, D), bf16),
        scratch_shapes=[
            pltpu.VMEM((F,), bf16),
            pltpu.VMEM((D,), bf16),
            pltpu.VMEM((TS, D), bf16),
            pltpu.VMEM((T - TS, D), bf16),
            pltpu.VMEM((T, D), bf16),
            pltpu.VMEM((D, 3 * D), bf16),
            pltpu.VMEM((D, D), bf16),
            pltpu.VMEM((3 * DH, 16, D), u32),
            pltpu.VMEM((DH, 16, D), u32),
            pltpu.VMEM((F, D), bf16),
            pltpu.VMEM((F, D), bf16),
            pltpu.VMEM((F // 2, D), u32),
            pltpu.VMEM((F // 2, D), u32),
            pltpu.VMEM((T, D), f32),
            pltpu.VMEM((T // 2, D), u32),
            pltpu.VMEM((NC, T, 128), f32),
            pltpu.VMEM((2, 2 * NC, HALO + T, 128), f32),
            pltpu.VMEM((T // 2, D), u32),
            pltpu.VMEM((T // 2, F), u32),
            pltpu.VMEM((W, T, 128), f32),
            pltpu.VMEM((W, T, 128), f32),
            pltpu.SemaphoreType.DMA((9,)),
        ],
        compiler_params=pltpu.CompilerParams(
            dimension_semantics=("arbitrary",),
            vmem_limit_bytes=64 * 1024 * 1024,
        ),
    )(A_x.reshape(S, D), A_wqkv, A_wo, B_w1.T, B_b1, B_w2, B_b2)
    return out.reshape(1, S, D)
```

```python
import jax
import jax.numpy as jnp
import jax.experimental.pallas as pl
import jax.experimental.pallas.tpu as pltpu

S, D, F = 2048, 512, 1376
H, DH, W, DIL = 32, 16, 8, 2
T = 512
TS = 128
RC = 16
LC = 32
NS = T // TS
NB = S // T
HALO = 16
EPS = 1e-5
NC = D // 128
f32 = jnp.float32
bf16 = jnp.bfloat16
u32 = jnp.uint32
NN = (((1,), (0,)), ((), ()))
NT = (((1,), (1,)), ((), ()))
LOG2E = 1.4426950408889634

ORDER = ("L1_Q0_Q1_L2_O0_Q2_O1_L3_Q3_O2_W_A1_A0_B1_B0_A2_O3_B2_q0_q1_q2_o0_A3_B3_a0_o1_q3_"
         "a1_o2_b1_b0_a2_o3_b2_N_a3_b3")
PRO = ("wq0_Pq0_wq1_X0_Pq1_Q0q_X1_wk_Pk_L1_Q1q_Q0k_wv_Pv_Q1k_Q1v_Q0v_t06_X2_wo_L2_t1_L3_Po_"
       "t0_Q2_O0_n0_O1_t2_n1_Q3_O2_t3")
CATT = 160
CLN = 100


def _ln(x):
    m = jnp.mean(x, axis=-1, keepdims=True)
    xc = x - m
    v = jnp.mean(xc * xc, axis=-1, keepdims=True)
    return xc * jax.lax.rsqrt(v + EPS)


def _gelu(x):
    c = 0.7978845608028654
    hx = 0.5 * x
    return hx + hx * jnp.tanh(x * (c + (c * 0.044715) * (x * x)))


def _pack(x):
    return pltpu.bitcast(x.astype(bf16), u32)


def _unpack(x):
    return pltpu.bitcast(x, bf16)


def _plan():
    tiles = {"Q": [TS] * (3 * NC), "O": [TS] * NC, "A": [TS // 2] * (-(-F // 128)),
             "B": [TS * 11 // 4] * NC}
    chunks = {"att": [CATT] * (TS // RC), "ln1": [CLN] * (TS // LC),
              "ln2": [2 * CLN] * (TS // LC), "lnx": [CLN] * (TS // LC)}
    plans = [[], []]
    cur = plans[0]
    queue = []
    credit = 0
    seen = []

    def emit(e):
        cur.append((e[1], e[2], e[3], e[4], False))
        e[4] += 1
        if e[4] == len(chunks[e[1]]):
            queue.remove(e)

    def flush(pred):
        for e in [e for e in queue if pred(e)]:
            while e in queue:
                emit(e)

    for tok in ORDER.split("_"):
        if tok == "W":
            flush(lambda e: e[1] == "lnx")
            cur = plans[1]
            continue
        if tok == "N":
            queue.append(["N", "lnx", 0, 0, 0])
            continue
        k, s = tok[0], int(tok[1])
        if k == "L":
            queue.append([s, "lnx", 0, s, 0])
            continue
        l = 1 if k.islower() else 0
        k = k.upper()
        first = all(e[0] != k for e in seen)
        seen.append((k, l, s))
        flush(lambda e: e[0] == s)
        for i, cost in enumerate(tiles[k]):
            cur.append((k, l, s, i, first))
            credit += cost
            while credit > 0:
                cand = [e for e in queue if not (e[1] == "att" and k == "B")]
                if not cand:
                    break
                credit -= chunks[cand[0][1]][0]
                emit(cand[0])
            credit = min(credit, 0)
        if k == "Q":
            queue.append([s, "att", l, s, 0])
        elif k == "O":
            queue.append([s, "ln2", l, s, 0])
        elif k == "B" and l == 0:
            queue.append([s, "ln1", 1, s, 0])
    flush(lambda e: True)
    assert len(set(seen)) == 8 * NS
    return plans


def _kernel(x_hbm, wqkv_hbm, wo_hbm, w1_hbm, b1_hbm, w2_hbm, b2_hbm, o_hbm,
            b1_ref, b2_ref, xf_ref, xr_ref, ob_ref, wraw_ref, woraw_ref, wt_ref, wop_ref,
            w1_ref, w2_ref, w1p_ref, w2p_ref,
            xs_ref, xn_ref, q_ref, kv_ref, a_ref, g_ref, l_ref, u_ref, sem):
    blk = pl.program_id(0)

    def xf_copy(b):
        return pltpu.make_async_copy(x_hbm.at[pl.ds(b * T, TS), :], xf_ref, sem.at[0])

    def xr_copy(b):
        return pltpu.make_async_copy(x_hbm.at[pl.ds(b * T + TS, T - TS), :], xr_ref, sem.at[1])

    x1_copy = pltpu.make_async_copy(x_hbm.at[pl.ds(TS, TS), :], xr_ref.at[pl.ds(0, TS), :], sem.at[1])
    x2_copy = pltpu.make_async_copy(x_hbm.at[pl.ds(2 * TS, T - 2 * TS), :],
                                    xr_ref.at[pl.ds(TS, T - 2 * TS), :], sem.at[2])

    def o_copy(b):
        return pltpu.make_async_copy(ob_ref.at[pl.ds(0, T - TS), :], o_hbm.at[pl.ds(b * T, T - TS), :],
                                     sem.at[2])

    def o2_copy(b):
        return pltpu.make_async_copy(ob_ref.at[pl.ds(T - TS, TS), pl.ds(D - 128, 128)],
                                     o_hbm.at[pl.ds(b * T + T - TS, TS), pl.ds(D - 128, 128)], sem.at[3])

    def o3_copy(b):
        return pltpu.make_async_copy(ob_ref.at[pl.ds(T - TS, TS), pl.ds(0, D - 128)],
                                     o_hbm.at[pl.ds(b * T + T - TS, TS), pl.ds(0, D - 128)], sem.at[4])

    def wqkv_copy(p, half=None):
        if half is None:
            return pltpu.make_async_copy(wqkv_hbm.at[:, pl.ds(p * D, D)], wraw_ref.at[:, pl.ds(p * D, D)],
                                         sem.at[4 + p])
        c0 = p * D + half * (D // 2)
        return pltpu.make_async_copy(wqkv_hbm.at[:, pl.ds(c0, D // 2)], wraw_ref.at[:, pl.ds(c0, D // 2)],
                                     sem.at[4 + p if half == 0 else 3])

    wo_copy = pltpu.make_async_copy(wo_hbm, woraw_ref, sem.at[7])
    late_copies = [pltpu.make_async_copy(src, dst, sem.at[8]) for src, dst in (
        (b1_hbm, b1_ref), (b2_hbm, b2_ref), (w1_hbm, w1_ref), (w2_hbm, w2_ref))]

    def rows(s):
        return slice(s * TS, (s + 1) * TS)

    def hrows(s):
        return slice(s * TS // 2, (s + 1) * TS // 2)

    row128 = jax.lax.broadcasted_iota(jnp.int32, (RC, 128), 0)

    def lnx(l, s, i, first, first_block):
        r0 = s * TS + i * LC
        x = (xf_ref[r0:r0 + LC, :] if s == 0 else xr_ref[r0 - TS:r0 - TS + LC, :]).astype(f32)
        xs_ref[r0:r0 + LC, :] = x
        xn_ref[r0 // 2:(r0 + LC) // 2, :] = _pack(_ln(x))

    def ln1(l, s, i, first, first_block):
        r0 = s * TS + i * LC
        xn_ref[r0 // 2:(r0 + LC) // 2, :] = _pack(_ln(xs_ref[r0:r0 + LC, :]))

    def ln2(l, s, i, first, first_block):
        r0 = s * TS + i * LC
        xn_ref[r0 // 2:(r0 + LC) // 2, :] = _pack(_ln(_ln(xs_ref[r0:r0 + LC, :])))

    def qkv(l, s, c, first, first_block):
        xn = _unpack(xn_ref[hrows(s), :])
        wt = _unpack(wt_ref[4 * c:4 * c + 4].reshape(64, D))
        rc = jax.lax.dot_general(xn, wt, NT, preferred_element_type=f32)
        if c < NC:
            q_ref[c, rows(s), :] = rc * LOG2E
        else:
            kv_ref[l, c - NC, HALO + s * TS:HALO + (s + 1) * TS, :] = rc

    def att(l, s, i, first, first_block):
        r0 = s * TS + i * RC
        q = [q_ref[c, r0:r0 + RC, :] for c in range(NC)]
        ls = []
        for w in range(W):
            b = HALO + r0 - DIL * w
            p = [q[c] * kv_ref[l, c, b:b + RC, :] for c in range(NC)]
            t = (p[0] + p[1]) + (p[2] + p[3])
            t = t + pltpu.roll(t, 64, 1)
            rr = pltpu.roll(t, 32, 1)
            u_ref[w, r0:r0 + RC, :] = t
            t = u_ref[w, r0:r0 + RC, :] + rr
            if r0 < DIL * w and first_block is not False:
                bad = row128 + r0 < DIL * w
                if first_block is not True:
                    bad = jnp.logical_and(bad, first_block)
                t = jnp.where(bad, -1e9, t)
            l_ref[w, r0:r0 + RC, :] = t
            ls.append(l_ref[w, r0:r0 + RC, :])
        mx = ls[0]
        for w in range(1, W):
            mx = jnp.maximum(mx, ls[w])
        es = [jnp.exp2(x - mx) for x in ls]
        den = es[0]
        for w in range(1, W):
            den = den + es[w]
        inv = pl.reciprocal(den, approx=True)
        inv = inv * (2.0 - den * inv)
        outs = []
        for c in range(NC):
            acc = None
            for w in range(W):
                b = HALO + r0 - DIL * w
                pv = es[w] * kv_ref[l, NC + c, b:b + RC, :]
                acc = pv if acc is None else acc + pv
            outs.append(acc * inv)
        a_ref[r0 // 2:(r0 + RC) // 2, :] = _pack(jnp.concatenate(outs, axis=1))

    def wo(l, s, c, first, first_block):
        cs = slice(c * 128, (c + 1) * 128)
        wj = _unpack(wop_ref[:, :, cs].reshape(D // 2, 128))
        r = jnp.dot(_unpack(a_ref[hrows(s), :]), wj, preferred_element_type=f32)
        xs_ref[rows(s), cs] = xs_ref[rows(s), cs] + r

    def bias(ref, n0, n1):
        return ref[n0:n1].astype(f32).reshape(1, n1 - n0)

    def w1(l, s, i, first, first_block):
        n0 = i * 128
        n1 = min(F, n0 + 128)
        y = _unpack(xn_ref[hrows(s), :])
        if first:
            wj = w1_ref[n0:n1, :]
            w1p_ref[n0 // 2:n1 // 2, :] = pltpu.bitcast(wj, u32)
        else:
            wj = _unpack(w1p_ref[n0 // 2:n1 // 2, :])
        if n1 - n0 < 128:
            h = jax.lax.dot_general(wj, y, NT, preferred_element_type=f32).T
        else:
            h = jax.lax.dot_general(y, wj, NT, preferred_element_type=f32)
        h = h + bias(b1_ref, n0, n1)
        g_ref[hrows(s), n0:n1] = _pack(_gelu(h))

    def w2(l, s, c, first, first_block):
        cs = slice(c * 128, (c + 1) * 128)
        if l == 1 and s == NS - 1 and c == 0:
            o_copy(blk).start()
        if l == 1 and s == NS - 1 and c == NC - 1:
            o3_copy(blk).start()
        if first:
            wj = w2_ref[:, cs]
            w2p_ref[:, cs] = pltpu.bitcast(wj, u32)
        else:
            wj = _unpack(w2p_ref[:, cs])
        r = xs_ref[rows(s), cs] + jnp.dot(_unpack(g_ref[hrows(s), :]), wj, preferred_element_type=f32) \
            + bias(b2_ref, c * 128, (c + 1) * 128)
        if l == 0:
            xs_ref[rows(s), cs] = r
        else:
            ob_ref[rows(s), cs] = r.astype(bf16)

    fns = {"Q": qkv, "O": wo, "A": w1, "B": w2, "att": att, "ln1": ln1, "ln2": ln2, "lnx": lnx}

    def run(items, first_block):
        for kind, l, s, i, first in items:
            fns[kind](l, s, i, first, first_block)

    plan1, plan2 = _plan()

    @pl.when(blk == 0)
    def _():
        wqkv_copy(0, 0).start()
        xf_copy(0).start()
        wqkv_copy(0, 1).start()
        x1_copy.start()
        wqkv_copy(1).start()
        wqkv_copy(2).start()
        x2_copy.start()
        wo_copy.start()
        for cp in late_copies:
            cp.start()
        kv_ref[:, :, 0:HALO, :] = jnp.zeros((2, 2 * NC, HALO, 128), f32)
        rho = jax.lax.broadcasted_iota(jnp.int32, (128, 128), 0)
        col = jax.lax.broadcasted_iota(jnp.int32, (128, 128), 1)
        hit = rho == (col % DH) * 8 + col // DH

        def permute(dst, p, scale, get, dims, pairs=(0, 1)):
            perm = jnp.where(hit, scale, 0.0).astype(bf16)
            for pair in pairs:
                o = [jax.lax.dot_general(perm, get(2 * pair + c), dims,
                                         preferred_element_type=f32).reshape(DH, 8, D) for c in range(2)]
                z = jnp.concatenate(o, axis=1).reshape(DH * 16, D)
                dst[p * DH:(p + 1) * DH, pair * 8:(pair + 1) * 8, :] = _pack(z).reshape(DH, 8, D)

        left = list(plan1)

        def take(tok):
            k, s = tok[0], int(tok[1])
            kind = {"t": "att", "n": "ln2", "L": "lnx"}.get(k, k)
            sel = [e for e in left if e[0] == kind and e[2] == s]
            if len(tok) > 2:
                if kind == "Q":
                    sel = [e for e in sel if e[3] // NC == "qkv".index(tok[2])]
                else:
                    sel = sel[:int(tok[2:])]
            for e in sel:
                left.remove(e)
            run(sel, True)

        for tok in PRO.split("_"):
            if tok[0] == "P" and tok[1] in "qkv":
                p = "qkv".index(tok[1])
                half = int(tok[2]) if len(tok) > 2 else None
                permute(wt_ref, p, DH ** -0.5 if p == 0 else 1.0,
                        lambda c: wraw_ref[:, (p * NC + c) * 128:(p * NC + c + 1) * 128], NT,
                        (0, 1) if half is None else (half,))
            elif tok[0] == "w" and tok[1] in "qkv":
                wqkv_copy("qkv".index(tok[1]), int(tok[2]) if len(tok) > 2 else None).wait()
            elif tok == "wo":
                wo_copy.wait()
            elif tok == "X0":
                xf_copy(0).wait()
                run([("lnx", 0, 0, i, False) for i in range(TS // LC)], True)
            elif tok == "Po":
                permute(wop_ref, 0, 1.0, lambda c: woraw_ref[c * 128:(c + 1) * 128, :], NN)
            elif tok == "X1":
                xf_copy(1).start()
                x1_copy.wait()
            elif tok == "X2":
                x2_copy.wait()
            else:
                take(tok)
        assert not left

    @pl.when(blk < NB - 1)
    def _():
        xr_copy(blk + 1).start()

    @pl.when(blk == 0)
    def _():
        for cp in late_copies:
            cp.wait()

    @pl.when(blk > 0)
    def _():
        o_copy(blk - 1).wait()
        o2_copy(blk - 1).wait()
        o3_copy(blk - 1).wait()

    @pl.when(blk < NB - 1)
    def _():
        xf_copy(blk + 1).wait()

    run(plan2, blk == 0)

    o2_copy(blk).start()

    @pl.when(blk < NB - 2)
    def _():
        xf_copy(blk + 2).start()

    @pl.when(blk < NB - 1)
    def _():
        xr_copy(blk + 1).wait()
        kv_ref[:, :, 0:HALO, :] = kv_ref[:, :, T:T + HALO, :]
        run(plan1, False)

    @pl.when(blk == NB - 1)
    def _():
        o_copy(blk).wait()
        o3_copy(blk).wait()
        o2_copy(blk).wait()


@jax.jit
def pallas_interleave_layers__sliding_local_dilated__mixer_channel_mlp__prompt_kernel(
    A_x: jax.Array,
    A_wqkv: jax.Array,
    A_wo: jax.Array,
    B_x: jax.Array,
    B_w1: jax.Array,
    B_b1: jax.Array,
    B_w2: jax.Array,
    B_b2: jax.Array,
):
    hbm = pl.BlockSpec(memory_space=pl.ANY)
    out = pl.pallas_call(
        _kernel,
        grid=(NB,),
        in_specs=[hbm] * 7,
        out_specs=hbm,
        out_shape=jax.ShapeDtypeStruct((S, D), bf16),
        scratch_shapes=[
            pltpu.VMEM((F,), bf16),
            pltpu.VMEM((D,), bf16),
            pltpu.VMEM((TS, D), bf16),
            pltpu.VMEM((T - TS, D), bf16),
            pltpu.VMEM((T, D), bf16),
            pltpu.VMEM((D, 3 * D), bf16),
            pltpu.VMEM((D, D), bf16),
            pltpu.VMEM((3 * DH, 16, D), u32),
            pltpu.VMEM((DH, 16, D), u32),
            pltpu.VMEM((F, D), bf16),
            pltpu.VMEM((F, D), bf16),
            pltpu.VMEM((F // 2, D), u32),
            pltpu.VMEM((F // 2, D), u32),
            pltpu.VMEM((T, D), f32),
            pltpu.VMEM((T // 2, D), u32),
            pltpu.VMEM((NC, T, 128), f32),
            pltpu.VMEM((2, 2 * NC, HALO + T, 128), f32),
            pltpu.VMEM((T // 2, D), u32),
            pltpu.VMEM((T // 2, F), u32),
            pltpu.VMEM((W, T, 128), f32),
            pltpu.VMEM((W, T, 128), f32),
            pltpu.SemaphoreType.DMA((9,)),
        ],
        compiler_params=pltpu.CompilerParams(
            dimension_semantics=("arbitrary",),
            vmem_limit_bytes=64 * 1024 * 1024,
        ),
    )(A_x.reshape(S, D), A_wqkv, A_wo, B_w1.T, B_b1, B_w2, B_b2)
    return out.reshape(1, S, D)
```
